```python
import os as _os
_os.environ.setdefault("JAX_PLATFORMS", "cpu")
import jax
import jax.numpy as jnp

def _softmax(x, axis=-1):
    return jax.nn.softmax(x, axis=axis)
def _gelu(x):
    return jax.nn.gelu(x, approximate=True)
def _silu(x):
    return jax.nn.silu(x)
def _sigmoid(x):
    return jax.nn.sigmoid(x)
def _layernorm(x, axis=-1, eps=1e-5):
    m = jnp.mean(x, axis=axis, keepdims=True)
    v = jnp.var(x, axis=axis, keepdims=True)
    return (x - m) / jnp.sqrt(v + eps)
def _scatter_add(tgt, idx, src, axis=0):
    return tgt.at[idx].add(src)
def _segment_sum(src, seg, n):
    return jax.ops.segment_sum(src, seg, n)
class _Rng:
    def __init__(self, key):
        self._k = key
    def _next(self):
        self._k, sub = jax.random.split(self._k)
        return sub
    def normal(self, shape):
        return jax.random.normal(self._next(), shape, dtype=jnp.bfloat16)
    def randint(self, lo, hi, shape):
        return jax.random.randint(self._next(), shape, lo, hi, dtype=jnp.int32)
    def uniform(self, shape, lo=0.0, hi=1.0):
        return jax.random.uniform(self._next(), shape, jnp.bfloat16, lo, hi)
    def permutation(self, n):
        return jax.random.permutation(self._next(), n)


kernel_name = 'standalone__instancenorm__sampling'

def setup_inputs():
    _rng = _Rng(jax.random.key(int.from_bytes(__import__("os").urandom(4), "little")))
    _w = (lambda a: (lambda t: t.astype(jnp.bfloat16) if jnp.issubdtype(t.dtype, jnp.floating) else t)(jnp.asarray(a)))
    B, C, H, W = 16, 640, 16, 32
    return {
        "x": _w((lambda *s: _rng.normal(s) * 0.05)(B, C, H, W)),
        "g": _w((lambda *s: _rng.normal(s) * 0.05)(C) + 1.0),
        "b": _w((lambda *s: _rng.normal(s) * 0.05)(C)),
    }

def reference(x, g, b):
    mu = x.mean(axis=(-2, -1), keepdims=True)
    var = ((x - mu) * (x - mu)).mean(axis=(-2, -1), keepdims=True)
    xhat = (x - mu) / jnp.sqrt(var + 1e-5)
    return xhat * g.reshape(1, -1, 1, 1) + b.reshape(1, -1, 1, 1)
```

```python
import jax
import jax.numpy as jnp
import jax.experimental.pallas as pl
import jax.experimental.pallas.tpu as pltpu


@jax.jit
def pallas_standalone__instancenorm__sampling_kernel(x, g, b):
    B, C, H, W = x.shape
    S = H * W
    xt = jnp.transpose(x, (0, 2, 3, 1)).reshape(B, S, C)

    def body(x_ref, g_ref, b_ref, o_ref):
        xv = x_ref[...].astype(jnp.float32)
        gv = g_ref[...].astype(jnp.float32).reshape(1, C)
        bv = b_ref[...].astype(jnp.float32).reshape(1, C)
        mu = jnp.mean(xv, axis=0, keepdims=True)
        d = xv - mu
        var = jnp.mean(d * d, axis=0, keepdims=True)
        sc = jax.lax.rsqrt(var + 1e-5) * gv
        o_ref[...] = (d * sc + bv).astype(o_ref.dtype)

    out = pl.pallas_call(
        body,
        grid=(B,),
        in_specs=[
            pl.BlockSpec((None, S, C), lambda i: (i, 0, 0)),
            pl.BlockSpec((C,), lambda i: (0,)),
            pl.BlockSpec((C,), lambda i: (0,)),
        ],
        out_specs=pl.BlockSpec((None, S, C), lambda i: (i, 0, 0)),
        out_shape=jax.ShapeDtypeStruct((B, S, C), x.dtype),
        compiler_params=pltpu.CompilerParams(dimension_semantics=("parallel",)),
    )(xt, g, b)
    return jnp.transpose(out.reshape(B, H, W, C), (0, 3, 1, 2))
```

```python
import jax
import jax.numpy as jnp
import jax.experimental.pallas as pl
import jax.experimental.pallas.tpu as pltpu

_EPS = 1e-5


def _normalize_item(buf, i, gv, bv):
    xv = buf[i].astype(jnp.float32)
    mu = jnp.mean(xv, axis=0, keepdims=True)
    d = xv - mu
    var = jnp.mean(d * d, axis=0, keepdims=True)
    sc = jax.lax.rsqrt(var + _EPS) * gv
    buf[i] = (d * sc + bv).astype(buf.dtype)


@jax.jit
def pallas_standalone__instancenorm__sampling_kernel(x, g, b):
    B, C, H, W = x.shape
    S = H * W
    xt = jnp.transpose(x, (0, 2, 3, 1)).reshape(B, S, C)

    RC = 32
    WC = 32
    G = 4
    RA = 4
    LAST = 1

    def body(x_hbm, g_hbm, b_hbm, o_hbm, buf, gbuf, bbuf, sems):
        def start_reads(lo, hi, s):
            n = 0
            for it in range(lo, hi):
                for j in range(S // 2 // RC):
                    for half in range(2):
                        r0 = half * (S // 2) + j * RC
                        sl = (pl.ds(it, 1), pl.ds(r0, RC))
                        pltpu.make_async_copy(x_hbm.at[sl], buf.at[sl], sems.at[s]).start(priority=n % 2)
                        n += 1

        def start_writes(lo, hi, s):
            for j in range(S // WC):
                sl = (pl.ds(lo, hi - lo), pl.ds(j * WC, WC))
                pltpu.make_async_copy(buf.at[sl], o_hbm.at[sl], sems.at[s]).start()

        def wait_items(lo, hi, s):
            r = buf.at[pl.ds(lo, hi - lo)]
            pltpu.make_async_copy(r, r, sems.at[s]).wait()

        def compute(lo, hi, gv, bv):
            def one(i, carry):
                _normalize_item(buf, i, gv, bv)
                return carry
            jax.lax.fori_loop(lo, hi, one, 0)

        gcp = pltpu.make_async_copy(g_hbm, gbuf, sems.at[0])
        bcp = pltpu.make_async_copy(b_hbm, bbuf, sems.at[0])
        gcp.start()
        bcp.start()
        start_reads(0, RA, 0)
        start_reads(RA, B - LAST, 1)
        start_reads(B - LAST, B, 2)
        gcp.wait()
        bcp.wait()
        wait_items(0, RA, 0)
        gv = gbuf[...].astype(jnp.float32).reshape(1, C)
        bv = bbuf[...].astype(jnp.float32).reshape(1, C)
        compute(0, RA, gv, bv)
        wait_items(RA, B - LAST, 1)
        start_writes(0, RA, 0)
        wait_items(B - LAST, B, 2)
        for lo in range(RA, B, G):
            compute(lo, lo + G, gv, bv)
            start_writes(lo, lo + G, 0)
        wait_items(0, B, 0)

    out = pl.pallas_call(
        body,
        in_specs=[pl.BlockSpec(memory_space=pl.ANY)] * 3,
        out_specs=pl.BlockSpec(memory_space=pl.ANY),
        out_shape=jax.ShapeDtypeStruct((B, S, C), x.dtype),
        scratch_shapes=[
            pltpu.VMEM((B, S, C), x.dtype),
            pltpu.VMEM((C,), g.dtype),
            pltpu.VMEM((C,), b.dtype),
            pltpu.SemaphoreType.DMA((3,)),
        ],
        compiler_params=pltpu.CompilerParams(vmem_limit_bytes=64 * 1024 * 1024),
    )(xt, g, b)
    return jnp.transpose(out.reshape(B, H, W, C), (0, 3, 1, 2))
```

```python
import jax
import jax.numpy as jnp
from jax import lax
import jax.experimental.pallas as pl
import jax.experimental.pallas.tpu as pltpu

_EPS = 1e-5
_ROWS = 32
_GROUPS = (6, 5, 5)
_TAIL_ITEMS = 4
_TAIL_ROWS = 160


def _normalize_item(buf, i, gv, bv):
    xv = buf[i].astype(jnp.float32)
    mu = jnp.mean(xv, axis=0, keepdims=True)
    d = xv - mu
    var = jnp.mean(d * d, axis=0, keepdims=True)
    scale = lax.rsqrt(var + _EPS) * gv
    buf[i] = (d * scale + bv).astype(buf.dtype)


@jax.jit
def pallas_standalone__instancenorm__sampling_kernel(
    x: jax.Array,
    g: jax.Array,
    b: jax.Array,
):
    B, C, H, W = x.shape
    S = H * W
    assert sum(_GROUPS) == B and S % _ROWS == 0 and _TAIL_ROWS % _ROWS == 0
    assert _TAIL_ROWS < S and _TAIL_ITEMS <= B - _GROUPS[0]
    first = _GROUPS[0]
    tail_lo = B - _TAIL_ITEMS
    tail_row = S - _TAIL_ROWS

    def body(x_hbm, g_hbm, b_hbm, o_hbm, buf, gbuf, bbuf, sems):
        def start_reads(b0, b1, r0, r1, s):
            def step(j, carry):
                row = pl.multiple_of(r0 + j * _ROWS, _ROWS)
                for n, item in enumerate(range(b0, b1)):
                    sl = (pl.ds(item, 1), pl.ds(row, _ROWS))
                    pltpu.make_async_copy(x_hbm.at[sl], buf.at[sl], sems.at[s]).start(priority=n % 2)
                return carry

            lax.fori_loop(0, (r1 - r0) // _ROWS, step, 0)

        def start_writes(b0, b1, s):
            def step(j, carry):
                sl = (pl.ds(b0, b1 - b0), pl.ds(pl.multiple_of(j * _ROWS, _ROWS), _ROWS))
                pltpu.make_async_copy(buf.at[sl], o_hbm.at[sl], sems.at[s]).start()
                return carry

            lax.fori_loop(0, S // _ROWS, step, 0)

        def wait_region(b0, b1, r0, r1, s):
            ref = buf.at[pl.ds(b0, b1 - b0), pl.ds(r0, r1 - r0)]
            pltpu.make_async_copy(ref, ref, sems.at[s]).wait()

        def normalize(b0, b1, gv, bv):
            def step(i, carry):
                _normalize_item(buf, i, gv, bv)
                return carry

            lax.fori_loop(b0, b1, step, 0)

        g_copy = pltpu.make_async_copy(g_hbm, gbuf, sems.at[0])
        b_copy = pltpu.make_async_copy(b_hbm, bbuf, sems.at[0])
        start_reads(0, first, 0, S, 0)
        g_copy.start()
        b_copy.start()
        start_reads(first, B, 0, tail_row, 1)
        start_reads(first, tail_lo, tail_row, S, 1)

        g_copy.wait()
        b_copy.wait()
        wait_region(0, first, 0, S, 0)
        gv = gbuf[...].astype(jnp.float32).reshape(1, C)
        bv = bbuf[...].astype(jnp.float32).reshape(1, C)
        normalize(0, first, gv, bv)

        start_reads(tail_lo, B, tail_row, S, 0)
        wait_region(first, tail_lo, 0, S, 1)
        wait_region(tail_lo, B, 0, tail_row, 1)
        start_writes(0, first, 1)
        wait_region(tail_lo, B, tail_row, S, 0)

        b0 = first
        for n_items in _GROUPS[1:]:
            normalize(b0, b0 + n_items, gv, bv)
            start_writes(b0, b0 + n_items, 1)
            b0 += n_items
        wait_region(0, B, 0, S, 1)

    xt = jnp.transpose(x, (0, 2, 3, 1)).reshape(B, S, C)
    out = pl.pallas_call(
        body,
        in_specs=[pl.BlockSpec(memory_space=pl.ANY)] * 3,
        out_specs=pl.BlockSpec(memory_space=pl.ANY),
        out_shape=jax.ShapeDtypeStruct((B, S, C), x.dtype),
        scratch_shapes=[
            pltpu.VMEM((B, S, C), x.dtype),
            pltpu.VMEM((C,), g.dtype),
            pltpu.VMEM((C,), b.dtype),
            pltpu.SemaphoreType.DMA((2,)),
        ],
        compiler_params=pltpu.CompilerParams(vmem_limit_bytes=64 * 1024 * 1024),
    )(xt, g, b)
    return jnp.transpose(out.reshape(B, H, W, C), (0, 3, 1, 2))
```
